```python
import os as _os
_os.environ.setdefault("JAX_PLATFORMS", "cpu")
import jax
import jax.numpy as jnp

def _softmax(x, axis=-1):
    return jax.nn.softmax(x, axis=axis)
def _gelu(x):
    return jax.nn.gelu(x, approximate=True)
def _silu(x):
    return jax.nn.silu(x)
def _sigmoid(x):
    return jax.nn.sigmoid(x)
def _layernorm(x, axis=-1, eps=1e-5):
    m = jnp.mean(x, axis=axis, keepdims=True)
    v = jnp.var(x, axis=axis, keepdims=True)
    return (x - m) / jnp.sqrt(v + eps)
def _scatter_add(tgt, idx, src, axis=0):
    return tgt.at[idx].add(src)
def _segment_sum(src, seg, n):
    return jax.ops.segment_sum(src, seg, n)
class _Rng:
    def __init__(self, key):
        self._k = key
    def _next(self):
        self._k, sub = jax.random.split(self._k)
        return sub
    def normal(self, shape):
        return jax.random.normal(self._next(), shape, dtype=jnp.bfloat16)
    def randint(self, lo, hi, shape):
        return jax.random.randint(self._next(), shape, lo, hi, dtype=jnp.int32)
    def uniform(self, shape, lo=0.0, hi=1.0):
        return jax.random.uniform(self._next(), shape, jnp.bfloat16, lo, hi)
    def permutation(self, n):
        return jax.random.permutation(self._next(), n)


kernel_name = 'standalone__mha_softmax__near_ridge'

def setup_inputs():
    _rng = _Rng(jax.random.key(int.from_bytes(__import__("os").urandom(4), "little")))
    _w = (lambda a: (lambda t: t.astype(jnp.bfloat16) if jnp.issubdtype(t.dtype, jnp.floating) else t)(jnp.asarray(a)))
    B, H, Sq, Sk, D = 8, 32, 384, 512, 128
    return {
        "q": _w((lambda *s: _rng.normal(s) * 0.4)(B, H, Sq, D)),
        "k": _w((lambda *s: _rng.normal(s) * 0.4)(B, H, Sk, D)),
        "v": _w((lambda *s: _rng.normal(s) * 0.05)(B, H, Sk, D)),
    }

def reference(q, k, v):
    scale = q.shape[-1] ** -0.5
    scores = jnp.einsum("bhqd,bhkd->bhqk", q, k) * scale
    p = _softmax(scores, axis=-1)
    return jnp.einsum("bhqk,bhkd->bhqd", p, v)
```

```python
import jax
import jax.numpy as jnp
from jax import lax
import jax.experimental.pallas as pl
import jax.experimental.pallas.tpu as pltpu

LOG2E = 1.4426950408889634

GROUPS = 8
CHUNKS = 4
RING = 8
UNITS_PER_ITER = 38
READ_STEPS = 25
LAST_UNITS = 8
WRITE_ROWS = 96
WRITES_PER_ITER = 17


def _attention_head(q, k, v, scale_log2e):
    s = lax.dot_general(q, k, (((1,), (1,)), ((), ())), preferred_element_type=jnp.float32)
    m = jnp.max(s, axis=-1, keepdims=True)
    p = jnp.exp2((s - m) * scale_log2e)
    l = jnp.sum(p, axis=-1, keepdims=True)
    o = jnp.dot(p.astype(v.dtype), v, preferred_element_type=jnp.float32)
    r = pl.reciprocal(l, approx=True)
    r = r * (2.0 - l * r)
    return o * r


@jax.jit
def pallas_standalone__mha_softmax__near_ridge_kernel(
    q: jax.Array,
    k: jax.Array,
    v: jax.Array,
):
    B, H, Sq, D = q.shape
    Sk = k.shape[2]
    G, C = GROUPS, CHUNKS
    steps = B * H // G
    rq, rk = Sq // C, Sk // C
    unit_rows = rq + 2 * rk
    step_units = C * G
    units = steps * step_units
    X, N1, L, W = UNITS_PER_ITER, READ_STEPS, LAST_UNITS, WRITES_PER_ITER
    first = units - X * N1 - L
    writes_per_step = Sq // WRITE_ROWS
    offsets = (0, rq, rq + rk)
    sizes = (rq, rk, rk)
    scale_log2e = D ** -0.5 * LOG2E

    def kernel(q_hbm, k_hbm, v_hbm, o_hbm, x_buf, o_buf, read_sems, write_sem):
        def read_units(u0, n, lo=0, hi=None, sem=None):
            for d in range(lo, 3 * n if hi is None else hi):
                j, t = divmod(d, 3)
                u = u0 + j
                w = (u & (G - 1)) * (C * steps) + (u >> 3)
                pltpu.make_async_copy(
                    (q_hbm, k_hbm, v_hbm)[t].at[pl.ds(pl.multiple_of(w * sizes[t], sizes[t]), sizes[t])],
                    x_buf.at[pl.ds(pl.multiple_of(u * unit_rows + offsets[t], 32), sizes[t])],
                    read_sems.at[(u >> 5) & (RING - 1) if sem is None else sem],
                ).start(priority=d % 2)

        def wait_units(u0, n, sem):
            start = u0 * unit_rows
            if not isinstance(start, int):
                start = pl.multiple_of(start, 32)
            x = x_buf.at[pl.ds(start, n * unit_rows)]
            pltpu.make_async_copy(x, x, read_sems.at[sem]).wait()

        def write(m):
            rows = pl.ds(pl.multiple_of(m * WRITE_ROWS, WRITE_ROWS), WRITE_ROWS)
            pltpu.make_async_copy(o_buf.at[:, rows], o_hbm.at[:, rows], write_sem).start()

        def load(i, g, t):
            base = i * (step_units * unit_rows)
            return jnp.concatenate(
                [
                    x_buf[pl.ds(pl.multiple_of(base + (c * G + g) * unit_rows + offsets[t], 32), sizes[t]), :]
                    for c in range(C)
                ],
                axis=0,
            )

        def compute(i, g):
            o = _attention_head(load(i, g, 0), load(i, g, 1), load(i, g, 2), scale_log2e)
            o_buf[g, pl.ds(pl.multiple_of(i * Sq, Sq), Sq), :] = o.astype(o_buf.dtype)

        @pl.loop(0, first // G)
        def _(n):
            read_units(n * G, G)

        read_units(first // G * G, first % G)

        @pl.loop(0, N1)
        def _(i):
            wait_units(i * step_units, step_units, i & (RING - 1))
            for g in range(G):
                compute(i, g)
                read_units(first + i * X, X, g * 3 * X // G, (g + 1) * 3 * X // G)

        read_units(units - L, L, sem=RING)
        for i in range(N1, steps - 1):
            wait_units(i * step_units, step_units, i % RING)
        wait_units(units - step_units, step_units - L, (steps - 1) % RING)

        @pl.loop(0, steps - N1)
        def _(j):
            for w in range(W):
                write(j * W + w)

            @pl.when(j == steps - N1 - 1)
            def _():
                wait_units(units - L, L, RING)

            for g in range(G):
                compute(N1 + j, g)

        for m in range((steps - N1) * W, steps * writes_per_step):
            write(m)
        pltpu.make_async_copy(o_buf, o_hbm, write_sem).wait()

    out = pl.pallas_call(
        kernel,
        in_specs=[pl.BlockSpec(memory_space=pl.ANY)] * 3,
        out_specs=pl.BlockSpec(memory_space=pl.ANY),
        out_shape=jax.ShapeDtypeStruct((G, steps * Sq, D), q.dtype),
        scratch_shapes=[
            pltpu.VMEM((units * unit_rows, D), q.dtype),
            pltpu.VMEM((G, steps * Sq, D), q.dtype),
            pltpu.SemaphoreType.DMA((RING + 1,)),
            pltpu.SemaphoreType.DMA(()),
        ],
        compiler_params=pltpu.CompilerParams(vmem_limit_bytes=126 * 1024 * 1024),
    )(q.reshape(-1, D), k.reshape(-1, D), v.reshape(-1, D))
    return out.reshape(B, H, Sq, D)
```

```python
import jax
import jax.numpy as jnp
import jax.experimental.pallas as pl
import jax.experimental.pallas.tpu as pltpu

LOG2E = 1.4426950408889634

LOG2_SEGMENTS = 3
SEGMENTS = 1 << LOG2_SEGMENTS
CHUNK_ROWS = 128
READ_STEPS = 25
READS_PER_STEP = (28, 38, 38)
LAST_READS = 24
WRITE_ROWS = 96
FIRST_WRITES = 5
WRITES_PER_STEP = 17


def _attention_head(q, k, v):
    s = jax.lax.dot_general(
        q, k, (((1,), (1,)), ((), ())), preferred_element_type=jnp.float32
    )
    m = jnp.max(s, axis=-1, keepdims=True)
    p = jnp.exp2((s - m) * (q.shape[-1] ** -0.5 * LOG2E))
    l = jnp.sum(p, axis=-1, keepdims=True)
    o = jnp.dot(p.astype(v.dtype), v, preferred_element_type=jnp.float32)
    r = pl.reciprocal(l, approx=True)
    return o * (r * (2.0 - l * r))


def _multiple_of(x, n):
    return x if isinstance(x, int) else pl.multiple_of(x, n)


@jax.jit
def pallas_standalone__mha_softmax__near_ridge_kernel(
    q: jax.Array,
    k: jax.Array,
    v: jax.Array,
):
    B, H, Sq, D = q.shape
    Sk = k.shape[2]
    heads = B * H
    steps = heads // SEGMENTS
    write_steps = steps - READ_STEPS

    head_chunks = [s // CHUNK_ROWS for s in (Sq, Sk, Sk)]
    step_chunks = [c * SEGMENTS for c in head_chunks]
    first_reads = [
        n * steps - x * READ_STEPS for n, x in zip(step_chunks, READS_PER_STEP)
    ]
    step_magic = [-(-(1 << 16) // n) for n in step_chunks]
    step_writes = Sq // WRITE_ROWS

    assert heads % SEGMENTS == 0 and Sq % WRITE_ROWS == 0
    assert Sq % CHUNK_ROWS == 0 and Sk % CHUNK_ROWS == 0
    assert LAST_READS <= min(step_chunks[2], READS_PER_STEP[2])
    for n, first, x, magic in zip(step_chunks, first_reads, READS_PER_STEP, step_magic):
        assert all(first + x * i >= n * (i + 1) for i in range(READ_STEPS))
        assert all((u * magic) >> 16 == u // n for u in range(n * steps))
    assert all(
        FIRST_WRITES + (j + 1) * WRITES_PER_STEP <= (READ_STEPS + j) * step_writes
        for j in range(write_steps)
    )

    def kernel(q_hbm, k_hbm, v_hbm, o_hbm, q_buf, k_buf, v_buf, o_buf, write_sem):
        srcs = (q_hbm, k_hbm, v_hbm)
        bufs = (q_buf, k_buf, v_buf)

        def write(m):
            rows = pl.ds(_multiple_of(m * WRITE_ROWS, WRITE_ROWS), WRITE_ROWS)
            pltpu.make_async_copy(
                o_buf.at[:, rows], o_hbm.at[:, rows], write_sem
            ).start()

        def load(t, i, g):
            parts = []
            for c in range(head_chunks[t]):
                u = i * step_chunks[t] + c * SEGMENTS + g
                rows = pl.ds(_multiple_of(u * CHUNK_ROWS, CHUNK_ROWS), CHUNK_ROWS)
                parts.append(bufs[t][rows, :])
            return jnp.concatenate(parts, axis=0)

        def compute(i, g):
            o = _attention_head(load(0, i, g), load(1, i, g), load(2, i, g))
            o_buf[g, pl.ds(_multiple_of(i * Sq, Sq), Sq), :] = o.astype(o_buf.dtype)

        def run(read_sems):

            def read(t, u0, j, queue, in_last_read_step=None):
                lead = u0 + j % SEGMENTS
                segment, block = lead & (SEGMENTS - 1), lead >> LOG2_SEGMENTS
                row = (segment * (head_chunks[t] * steps) + block) * CHUNK_ROWS
                row += j // SEGMENTS * CHUNK_ROWS
                sem = ((u0 + j) * step_magic[t]) >> 16
                if in_last_read_step is not None:
                    sem = jnp.where(in_last_read_step, steps, sem)
                src = pl.ds(_multiple_of(row, CHUNK_ROWS), CHUNK_ROWS)
                row = u0 * CHUNK_ROWS + j * CHUNK_ROWS
                dst = pl.ds(_multiple_of(row, CHUNK_ROWS), CHUNK_ROWS)
                pltpu.make_async_copy(
                    srcs[t].at[src], bufs[t].at[dst], read_sems.at[t, sem]
                ).start(priority=queue)

            def read_all(starts, counts):
                order = [(t, j) for t in range(3) for j in range(counts[t])]
                for d, (t, j) in enumerate(order):
                    read(t, starts[t], j, d % 2)

            def wait(t, u0, n, sem):
                rows = pl.ds(_multiple_of(u0 * CHUNK_ROWS, CHUNK_ROWS), n * CHUNK_ROWS)
                filled = bufs[t].at[rows]
                pltpu.make_async_copy(filled, filled, read_sems.at[t, sem]).wait()

            def wait_step(i):
                for t in range(3):
                    wait(t, i * step_chunks[t], step_chunks[t], i)

            whole = min(f // n for f, n in zip(first_reads, step_chunks))

            @pl.loop(0, whole)
            def _(i):
                read_all([i * n for n in step_chunks], step_chunks)

            read_all(
                [whole * n for n in step_chunks],
                [f - whole * n for f, n in zip(first_reads, step_chunks)],
            )

            @pl.loop(0, READ_STEPS)
            def _(i):
                wait_step(i)
                order = [(t, j) for t in range(3) for j in range(READS_PER_STEP[t])]
                for g in range(SEGMENTS):
                    compute(i, g)
                    lo = g * len(order) // SEGMENTS
                    hi = (g + 1) * len(order) // SEGMENTS
                    for d in range(lo, hi):
                        t, j = order[d]
                        last = t == 2 and j >= READS_PER_STEP[t] - LAST_READS
                        read(
                            t,
                            first_reads[t] + i * READS_PER_STEP[t],
                            j,
                            d % 2,
                            i == READ_STEPS - 1 if last else None,
                        )

            for i in range(READ_STEPS, steps - 1):
                wait_step(i)
            for t in range(3):
                n = step_chunks[t] - (LAST_READS if t == 2 else 0)
                wait(t, (steps - 1) * step_chunks[t], n, steps - 1)

            for m in range(FIRST_WRITES):
                write(m)

            @pl.loop(0, write_steps)
            def _(j):
                for w in range(WRITES_PER_STEP):
                    write(FIRST_WRITES + j * WRITES_PER_STEP + w)

                @pl.when(j == write_steps - 1)
                def _():
                    wait(2, steps * step_chunks[2] - LAST_READS, LAST_READS, steps)

                for g in range(SEGMENTS):
                    compute(READ_STEPS + j, g)

        pl.run_scoped(run, pltpu.SemaphoreType.DMA((3, steps + 1)))

        issued = FIRST_WRITES + write_steps * WRITES_PER_STEP
        for m in range(issued, steps * step_writes):
            write(m)
        pltpu.make_async_copy(o_buf, o_hbm, write_sem).wait()

    out = pl.pallas_call(
        kernel,
        in_specs=[pl.BlockSpec(memory_space=pl.ANY)] * 3,
        out_specs=pl.BlockSpec(memory_space=pl.ANY),
        out_shape=jax.ShapeDtypeStruct((SEGMENTS, steps * Sq, D), q.dtype),
        scratch_shapes=[
            pltpu.VMEM((heads * Sq, D), q.dtype),
            pltpu.VMEM((heads * Sk, D), k.dtype),
            pltpu.VMEM((heads * Sk, D), v.dtype),
            pltpu.VMEM((SEGMENTS, steps * Sq, D), q.dtype),
            pltpu.SemaphoreType.DMA(()),
        ],
        compiler_params=pltpu.CompilerParams(vmem_limit_bytes=126 * 1024 * 1024),
    )(q.reshape(-1, D), k.reshape(-1, D), v.reshape(-1, D))
    return out.reshape(B, H, Sq, D)
```
